```python
import os as _os
_os.environ.setdefault("JAX_PLATFORMS", "cpu")
import jax
import jax.numpy as jnp

def _softmax(x, axis=-1):
    return jax.nn.softmax(x, axis=axis)
def _gelu(x):
    return jax.nn.gelu(x, approximate=True)
def _silu(x):
    return jax.nn.silu(x)
def _sigmoid(x):
    return jax.nn.sigmoid(x)
def _layernorm(x, axis=-1, eps=1e-5):
    m = jnp.mean(x, axis=axis, keepdims=True)
    v = jnp.var(x, axis=axis, keepdims=True)
    return (x - m) / jnp.sqrt(v + eps)
def _scatter_add(tgt, idx, src, axis=0):
    return tgt.at[idx].add(src)
def _segment_sum(src, seg, n):
    return jax.ops.segment_sum(src, seg, n)
class _Rng:
    def __init__(self, key):
        self._k = key
    def _next(self):
        self._k, sub = jax.random.split(self._k)
        return sub
    def normal(self, shape):
        return jax.random.normal(self._next(), shape, dtype=jnp.bfloat16)
    def randint(self, lo, hi, shape):
        return jax.random.randint(self._next(), shape, lo, hi, dtype=jnp.int32)
    def uniform(self, shape, lo=0.0, hi=1.0):
        return jax.random.uniform(self._next(), shape, jnp.bfloat16, lo, hi)
    def permutation(self, n):
        return jax.random.permutation(self._next(), n)


kernel_name = 'interleave_layers__spectral_gfnet__glu_gated_bilinear__prompt'

def setup_inputs():
    _rng = _Rng(jax.random.key(int.from_bytes(__import__("os").urandom(4), "little")))
    _w = (lambda a: (lambda t: t.astype(jnp.bfloat16) if jnp.issubdtype(t.dtype, jnp.floating) else t)(jnp.asarray(a)))
    def _A_setup():
        B, S, D = 1, 2048, 512
        Df = D // 2 + 1
        return {
            "x": _w((lambda *s: _rng.normal(s) * 0.05)(B, S, D)),
            "w_r": _w((lambda *s: _rng.normal(s) * 0.2)(S, Df) * 0.02),
            "w_i": _w((lambda *s: _rng.normal(s) * 0.2)(S, Df) * 0.02),
        }
    _A_in = _A_setup()

    def _B_setup():
        B, S, D, F = 1, 2048, 512, 1792
        return {
            "x": _w((lambda *s: _rng.normal(s) * 0.05)(B, S, D)),
            "w_gate": _w((lambda *s: _rng.normal(s) * 0.2)(D, F) * (D ** -0.5)),
            "w_up": _w((lambda *s: _rng.normal(s) * 0.2)(D, F) * (D ** -0.5)),
            "w_down": _w((lambda *s: _rng.normal(s) * 0.2)(F, D) * (F ** -0.5)),
        }
    _B_in = _B_setup()

    return {
        "A_x": _A_in["x"],
        "A_w_r": _A_in["w_r"],
        "A_w_i": _A_in["w_i"],
        "B_x": _B_in["x"],
        "B_w_gate": _B_in["w_gate"],
        "B_w_up": _B_in["w_up"],
        "B_w_down": _B_in["w_down"],
    }

def reference(A_x, A_w_r, A_w_i, B_x, B_w_gate, B_w_up, B_w_down):
    def _A_ref(x, w_r, w_i):
        B, S, D = x.shape
        X = (lambda x, axes=(-2,-1): jnp.fft.rfft2(x.astype(jnp.float32), axes=axes))(x, axes=(-2, -1))
        W = w_r + 1j * w_i
        X = X * W
        y = (lambda x, s, axes=(-2,-1): jnp.fft.irfft2(x, s=s, axes=axes).astype(jnp.bfloat16))(X, (S, D), axes=(-2, -1))
        return y

    def _B_ref(x, w_gate, w_up, w_down):
        g = jnp.einsum("bsd,df->bsf", x, w_gate)
        u = jnp.einsum("bsd,df->bsf", x, w_up)
        h = g * u
        return jnp.einsum("bsf,fd->bsd", h, w_down)

    x = A_x
    x = x + _A_ref(_layernorm(x, axis=-1), A_w_r, A_w_i)
    x = x + _B_ref(_layernorm(x, axis=-1), B_w_gate, B_w_up, B_w_down)
    x = x + _A_ref(_layernorm(x, axis=-1), A_w_r, A_w_i)
    x = x + _B_ref(_layernorm(x, axis=-1), B_w_gate, B_w_up, B_w_down)
    return x
```

```python
import math

import ml_dtypes
import numpy as np
import jax
import jax.numpy as jnp
from jax import lax
from jax.experimental import pallas as pl
from jax.experimental.pallas import tpu as pltpu

BF = ml_dtypes.bfloat16
EPS = 1e-5
S, D, F = 2048, 512, 1792
NT, TM = 8, 256
FC = 256
NCH = F // FC
HB = F // 2
WSPLIT = 3
f32, bf16, i32, u32 = jnp.float32, jnp.bfloat16, jnp.int32, jnp.uint32

POS_C = [0, 1, 2, 3, 4, 5, 6, 7, 8, 8, 9, 9]
POS_A = [2, 5, 8, 11, 11, 12, 12, 13, 14, 14, 15, 16, 16, 17, 18, 18]
PINC = (0, 1, 2, 3)
GSPLIT = 8

I_M0, I_M2, I_P = 0, 1, 2
I_N0, I_N2, I_C128, I_S128, I_F16 = 0, 1, 2, 3, 4


def build_consts():
    d2 = np.arange(128)[:, None].astype(np.float64)

    def cs(l):
        ph = 2*np.pi*((d2*np.asarray(l)[None, :]) % 512)/512.0
        return np.cos(ph), np.sin(ph)
    m = np.arange(32)
    M0 = np.zeros((128, 128)); M2 = np.zeros((128, 128))
    co, si = cs(4*m);        M0[:, 4*m+0] = co; M0[:, 4*m+1] = -si
    M0[:, 1] = (-1.0)**np.arange(128)
    co, si = cs(128+4*m);    M0[:, 4*m+2] = co; M0[:, 4*m+3] = -si
    co, si = cs(4*m+2);      M2[:, 4*m+2] = co; M2[:, 4*m+3] = -si
    co, si = cs(128+4*m+2);  M2[:, (4*m+4) % 128] = co; M2[:, (4*m+5) % 128] = -si
    M1 = np.zeros((256, 256))
    t = np.arange(1, 128, 2)

    def odd_cols(l):
        co, si = cs(l)
        sg = np.where(l % 4 == 1, 1.0, -1.0)[None, :]
        return np.concatenate([co, -sg*si], axis=0), np.concatenate([-si, -sg*co], axis=0)
    re, im = odd_cols(t);      M1[:, t] = re;                 M1[:, (t+1) % 128] = im
    re, im = odd_cols(128+t);  M1[:, 128+(t+2) % 128] = re;   M1[:, 128+(t+3) % 128] = im
    sc = 1.0/(S*D)
    N0 = np.zeros((128, 128)); N2 = np.zeros((128, 128)); N1 = np.zeros((256, 256))

    def inv_rows(l, cl):
        co, si = cs(l)
        return (cl*co).T*sc, (-cl*si).T*sc
    cl0 = np.where(4*m == 0, 1.0, 2.0)[None, :]
    r_, i_ = inv_rows(4*m, cl0);       N0[4*m+0] = r_; N0[4*m+1] = i_
    N0[1] = (-1.0)**np.arange(128)*sc
    r_, i_ = inv_rows(128+4*m, 2.0);   N0[4*m+2] = r_; N0[4*m+3] = i_
    r_, i_ = inv_rows(4*m+2, 2.0);     N2[4*m+2] = r_; N2[4*m+3] = i_
    r_, i_ = inv_rows(128+4*m+2, 2.0); N2[(4*m+4) % 128] = r_; N2[(4*m+5) % 128] = i_

    def odd_rows(l):
        co, si = cs(l)
        sg = np.where(l % 4 == 1, 1.0, -1.0)[None, :]
        return (np.concatenate([2*co, -2*sg*si], axis=0).T*sc,
                np.concatenate([-2*si, -2*sg*co], axis=0).T*sc)
    re, im = odd_rows(t);      N1[t] = re;               N1[(t+1) % 128] = im
    re, im = odd_rows(128+t);  N1[128+(t+2) % 128] = re; N1[128+(t+3) % 128] = im
    a = np.arange(128)
    ph = 2*np.pi*((a[:, None]*a[None, :]) % 128)/128.0
    C128, S128 = np.cos(ph), np.sin(ph)
    sa = np.arange(16)[:, None]; kl = np.arange(128)[None, :]
    ph = 2*np.pi*(sa*kl)/2048.0
    tw = np.stack([np.cos(ph), np.sin(ph)]).astype(np.float32)
    b = np.arange(16)
    ph = 2*np.pi*((b[:, None]*b[None, :]) % 16)/16.0
    C, Sn = np.cos(ph), np.sin(ph)
    F16 = np.zeros((128, 128))
    F16[0:32, 0:32] = np.block([[C, Sn], [-Sn, C]]); F16[32:64, 0:32] = np.block([[C, -Sn], [Sn, C]])
    P = np.zeros((128, 128))
    for a_ in range(8):
        for k2lo in range(4):
            for k1lo in range(4):
                P[16*a_+4*k2lo+k1lo, 32*k2lo+4*a_+k1lo] = 1.0
    d3 = np.arange(64).astype(np.float64)
    Q = {1: np.zeros((128, 128)), -1: np.zeros((128, 128))}
    for lp in range(1, 256, 2):
        l, sg = (lp, 1.0) if lp % 4 == 1 else (512 - lp, -1.0)
        ph = 2*np.pi*((d3*l) % 512)/512.0
        co, si = np.cos(ph), np.sin(ph)
        t_ = lp % 128 + (0 if lp < 128 else 4)
        Qc = Q[1 if l % 8 == 1 else -1]
        Qc[:, t_ % 128] = np.concatenate([co, -si])
        Qc[:, (t_+1) % 128] = sg*np.concatenate([-si, -co])

    def pack(a):
        u = np.ascontiguousarray(a).view(np.uint16).astype(np.uint32)
        return (u[..., 0::2, :] | (u[..., 1::2, :] << 16)).astype(np.uint32)
    c1 = np.stack([M0, M2, P]).astype(BF)
    c2 = np.stack([N0, N2, C128, S128, F16]).astype(BF)
    q4 = np.stack([Q[1], Q[-1], 2*sc*Q[1].T, 2*sc*Q[-1].T]).astype(BF)
    pm1 = pack(M1.astype(BF)); pn1 = pack(N1.astype(BF))
    cm = np.concatenate([pack(c1).reshape(192, 128), pm1[:, :128], pm1[:, 128:]], axis=0)
    cn = np.concatenate([pack(c2).reshape(320, 128), pn1[:, :128], pn1[:, 128:],
                         tw.reshape(32, 128).view(np.uint32), pack(q4).reshape(256, 128)], axis=0)
    return cm, cn


def _ub(v):
    return pltpu.bitcast(v, bf16)


def _dot(a, b):
    return jnp.dot(a, b, preferred_element_type=f32)


def cmul_const(v, num, den):
    re, im = v
    n = num % den
    if n == 0: return (re, im)
    if 4*n == den: return (im, -re)
    if 2*n == den: return (-re, -im)
    if 4*n == 3*den: return (-im, re)
    c = math.cos(2*math.pi*n/den); s = -math.sin(2*math.pi*n/den)
    if (8*n) % den == 0:
        r = math.sqrt(0.5)
        sc = 1.0 if c > 0 else -1.0; ss = 1.0 if s > 0 else -1.0
        a = (re - im) if sc*ss > 0 else (re + im)
        b = (re + im) if sc*ss > 0 else (im - re)
        return (a*(sc*r), b*(sc*r))
    return (re*c - im*s, re*s + im*c)


def cadd(a, b): return (a[0]+b[0], a[1]+b[1])
def csub(a, b): return (a[0]-b[0], a[1]-b[1])


def fft_list(v, sign):
    n = len(v)
    if n == 2: return [cadd(v[0], v[1]), csub(v[0], v[1])]
    if n == 4:
        a = cadd(v[0], v[2]); b = csub(v[0], v[2]); c = cadd(v[1], v[3]); d = csub(v[1], v[3])
        dj = (d[1], -d[0]) if sign > 0 else (-d[1], d[0])
        return [cadd(a, c), cadd(b, dj), csub(a, c), csub(b, dj)]
    e = fft_list(v[0::2], sign); o = fft_list(v[1::2], sign)
    out = [None]*n
    for k in range(n//2):
        t = cmul_const(o[k], sign*k, n)
        out[k] = cadd(e[k], t); out[k+n//2] = csub(e[k], t)
    return out


def layernorm(x):
    m = jnp.mean(x, axis=-1, keepdims=True)
    xc = x - m
    v = jnp.mean(xc*xc, axis=-1, keepdims=True)
    return xc * lax.rsqrt(v + EPS)


def ln_stats(x):
    s1 = jnp.sum(x, axis=-1, keepdims=True)
    s2 = jnp.sum(x*x, axis=-1, keepdims=True)
    m = s1 * (1.0/D)
    v = jnp.maximum(s2 * (1.0/D) - m*m, 0.0)
    return s1, m, lax.rsqrt(v + EPS)


def layernorm1(x):
    _, m, r = ln_stats(x)
    return x*r - m*r


def run(gen):
    for _ in gen: pass


def mix(*gens):
    alive = list(gens)
    while alive:
        for g in list(alive):
            if next(g, 'end') == 'end': alive.remove(g)


def interleave(main, nmain, sides):
    st = [[g, list(p), 0] for g, p in sides]

    def emit(step):
        for e in st:
            while e[2] < len(e[1]) and e[1][e[2]] <= step:
                next(e[0], None)
                e[2] += 1
    emit(-1)
    for i in range(nmain):
        next(main)
        emit(i)
    for _ in main: pass
    for e in st:
        for _ in e[0]: pass


def kernel(x_hbm, wr_hbm, wi_hbm, wg_hbm, wu_hbm, wd_hbm, cm_hbm, cn_hbm,
           out_hbm,
           xin, xs, xa, zb, wt, wtab, wn, wg, wu, wd, cm, cn, gm, obuf, tbuf, vbuf, rbuf, outb,
           midc, mida, yb, midp, gt,
           sx, sc, sw, sb, so):
    lane = lax.broadcasted_iota(i32, (64, 128), 1)
    odd = (lane & 1) == 1
    lo = (lane & 3) < 2
    lane8 = lax.broadcasted_iota(i32, (8, 128), 1)
    lo64 = lane < 64
    l8 = lane & 7
    mG = (l8 <= 2) | (l8 == 7)
    RS2 = math.sqrt(0.5)

    def aligned(j, k):
        return k*j if isinstance(j, int) else pl.multiple_of(k*j, k)

    def x_copy(j):
        return pltpu.make_async_copy(x_hbm.at[:, pl.ds(aligned(j, 8), 8), :], xin.at[j], sx.at[j])
    ccm = pltpu.make_async_copy(cm_hbm, cm, sc.at[0])
    ccn = pltpu.make_async_copy(cn_hbm, cn, sc.at[1])

    def w_copy(p, q):
        o = aligned(q, 512)
        return pltpu.make_async_copy((wr_hbm, wi_hbm)[p].at[:, pl.ds(o, 512)], wt.at[p, :, pl.ds(o, 512)],
                                     sw.at[2*q+p])

    def bg_copy(h, which):
        o = HB*h if isinstance(h, int) else pl.multiple_of(HB*h, 128)
        if which == 0:
            return pltpu.make_async_copy(wg_hbm.at[:, pl.ds(o, HB)], wg.at[:, pl.ds(o, HB)], sb.at[3*h])
        if which == 1:
            return pltpu.make_async_copy(wu_hbm.at[:, pl.ds(o, HB)], wu.at[:, pl.ds(o, HB)], sb.at[3*h+1])
        return pltpu.make_async_copy(wd_hbm.at[pl.ds(o, HB), :], wd.at[pl.ds(o, HB), :], sb.at[3*h+2])

    def o_copy(j, g):
        return pltpu.make_async_copy(outb.at[j, g], out_hbm.at[:, g, pl.ds(aligned(j, 8), 8), :], so.at[4*j+g])

    def c1(i): return _ub(cm[64*i:64*(i+1), :])
    def m1(): return jnp.concatenate([_ub(cm[192:320, :]), _ub(cm[320:448, :])], axis=1)
    def c2(i): return _ub(cn[64*i:64*(i+1), :])
    def n1(): return jnp.concatenate([_ub(cn[320:448, :]), _ub(cn[448:576, :])], axis=1)
    def q4(i): return _ub(cn[608+64*i:608+64*(i+1), :])
    def tw(i): return pltpu.bitcast(cn[576+16*i:576+16*(i+1), :], f32)

    x_copy(0).start()
    ccm.start()

    def _sx(j, _):
        x_copy(j).start(); return 0
    lax.fori_loop(1, NT, _sx, 0)

    def _sw(q, _):
        w_copy(0, q).start(); w_copy(1, q).start(); return 0
    lax.fori_loop(0, 4, _sw, 0)
    ccn.start()

    def _sb(h, _):
        for w in range(3): bg_copy(h, w).start()
        return 0
    lax.fori_loop(0, 2, _sb, 0)

    def ggen_tables():
        r64 = lax.broadcasted_iota(i32, (64, 128), 0); c64 = lax.broadcasted_iota(i32, (64, 128), 1)
        s2c = 8*(c64 >> 4) + (c64 & 7)
        pc0 = ((c64 >> 3) & 1) == 0
        th = ((r64*s2c) & 63).astype(f32) * (2*math.pi/64)
        c0 = jnp.cos(th); s0 = jnp.sin(th)
        gt[0] = jnp.where(pc0, c0, s0); gt[1] = jnp.where(pc0, -s0, c0)
        k1r = lax.broadcasted_iota(i32, (32, 128), 0); c32 = lax.broadcasted_iota(i32, (32, 128), 1)
        ph = (k1r*(8*(c32 >> 4) + (c32 & 7))).astype(f32) * (2*math.pi/2048)
        gt[2, 0:32] = jnp.cos(ph); gt[2, 32:64] = jnp.sin(ph)

    def ggen_part(lo_, hi_):
        A0t = gt[0]; A0b = gt[1]
        for k1 in range(lo_, hi_):
            cv = gt[2, k1:k1+1]; sv = gt[2, 32+k1:33+k1]
            gm[k1, 0:64, :] = (A0t*cv + A0b*sv).astype(bf16)
            gm[k1, 64:128, :] = (A0b*cv - A0t*sv).astype(bf16)

    ggen_tables()
    ggen_part(0, GSPLIT)
    vbuf[...] = jnp.zeros(vbuf.shape, f32)

    def fwd_gen(j, load_grp, post, p4, gp):
        vt = jnp.zeros((8, 128), f32)
        cat = lambda l: l[0] if len(l) == 1 else jnp.concatenate(l, axis=0)
        for g0 in range(0, 4, gp):
            ins = []; sts = []
            for g in range(g0, g0+gp):
                x = load_grp(g)
                if post:
                    sx_, _, r = ln_stats(x); sts.append((sx_, r))
                else:
                    x = layernorm(x)
                z0, z1, z2, z3 = [x[:, 128*i:128*(i+1)] for i in range(4)]
                a = z0+z2; b = z0-z2; c = z1+z3; dd = z1-z3
                y0 = (a+c).astype(bf16); y2 = (a-c).astype(bf16)
                if p4:
                    T1 = jnp.where(lo64, b, pltpu.roll(dd, 64, 1))
                    T2 = jnp.where(lo64, pltpu.roll(b-dd, 64, 1), b+dd) * RS2
                    ins.append((y0, y2, (T1+T2).astype(bf16), (T1-T2).astype(bf16)))
                else:
                    ins.append((y0, y2, jnp.concatenate([b, dd], axis=1).astype(bf16)))
                yield
            P0 = _dot(cat([t[0] for t in ins]), c1(I_M0)); P2 = _dot(cat([t[1] for t in ins]), c1(I_M2))
            if p4:
                PP = _dot(cat([t[2] for t in ins]), q4(0)); PM = _dot(cat([t[3] for t in ins]), q4(1))
            else:
                OO = _dot(cat([t[2] for t in ins]), m1())
            for g in range(g0, g0+gp):
                sl = slice(64*(g-g0), 64*(g-g0+1))
                p0, p2 = P0[sl], P2[sl]
                E_ = jnp.where(lo, p0, p2); Fm = jnp.where(lo, p2, p0)
                if p4:
                    Pp, Pm = PP[sl], PM[sl]
                    G_ = jnp.where(mG, Pp, Pm); H_ = jnp.where(mG, Pm, Pp)
                    ReA = jnp.where(odd, G_, E_)
                    ImA = pltpu.roll(jnp.where(odd, E_, G_), 127, 1)
                    H4 = pltpu.roll(H_, 124, 1); F2 = pltpu.roll(Fm, 126, 1)
                    ReB = jnp.where(odd, H4, F2)
                    ImB = pltpu.roll(jnp.where(odd, F2, H4), 127, 1)
                else:
                    O1, O2 = OO[sl, :128], OO[sl, 128:]
                    ReA = jnp.where(odd, O1, E_)
                    ImA = pltpu.roll(jnp.where(odd, E_, O1), 127, 1)
                    ReB = pltpu.roll(jnp.where(odd, O2, Fm), 126, 1)
                    ImB = pltpu.roll(jnp.where(odd, Fm, O2), 125, 1)
                if post:
                    sx_, r = sts[g-g0]
                    ReA = (ReA - jnp.where(lane == 0, sx_, 0.0)) * r
                    ImA = ImA * r; ReB = ReB * r; ImB = ImB * r
                for i in range(8):
                    s1 = g + 4*i
                    blk = ImA[8*i:8*i+8]
                    vt = jnp.where(lane8 == 4*s1, pltpu.roll(blk, 4*s1, 1) if s1 else blk, vt)
                ImA = jnp.where(lane == 0, 0.0, ImA)
                for lb, (re, im) in enumerate(((ReA, ImA), (ReB, ImB))):
                    r = fft_list([(re[8*i:8*i+8], im[8*i:8*i+8]) for i in range(8)], +1)
                    for kp in range(8):
                        t = cmul_const(r[kp], kp*g, 32)
                        midc[0, lb, kp, g] = t[0]; midc[1, lb, kp, g] = t[1]
                yield
        vt = pltpu.roll(vt, j >> 1, 1)
        h = j & 1
        vbuf[h] = jnp.where((lane8 & 3) == (j >> 1), vt, vbuf[h])
        r0 = aligned(j, 16)
        for kp in range(8):
            outs = [fft_list([(midc[0, lb, kp, g], midc[1, lb, kp, g]) for g in range(4)], +1) for lb in range(2)]
            for kq in range(4):
                re = jnp.concatenate([outs[0][kq][0], outs[1][kq][0]], axis=1)
                im = jnp.concatenate([outs[0][kq][1], outs[1][kq][1]], axis=1)
                obuf[kp+8*kq, pl.ds(r0, 16), :] = jnp.concatenate([re, im], axis=0).astype(bf16)
            if kp % 2 == 1: yield

    def inv_gen(j, load_grp, slot, late):
        p4 = not late
        r0 = aligned(j, 16)
        for b in range(8):
            ts = [tbuf[8*a+b, pl.ds(r0, 16), :].astype(f32) for a in range(4)]
            for lb in range(2):
                r = fft_list([(t[:8, 128*lb:128*(lb+1)], t[8:, 128*lb:128*(lb+1)]) for t in ts], -1)
                for g in range(4):
                    t = cmul_const(r[g], -g*b, 32)
                    mida[0, lb, b, g] = t[0]; mida[1, lb, b, g] = t[1]
            if b % 2 == 1 or late: yield

        def get_rt():
            rt = rbuf[j & 1]
            if isinstance(j, int):
                if j >> 1: rt = pltpu.roll(rt, 128 - (j >> 1), 1)
            else:
                rt = pltpu.roll(rt, (128 - (j >> 1)) & 127, 1)
            return rt
        if not late: rt = get_rt()
        for g in range(4):
            res = []
            for lb in range(2):
                r = fft_list([(mida[0, lb, b, g], mida[1, lb, b, g]) for b in range(8)], -1)
                res.append((jnp.concatenate([r[i][0] for i in range(8)], axis=0),
                            jnp.concatenate([r[i][1] for i in range(8)], axis=0)))
            (ReA, ImA), (ReB, ImB) = res
            if late:
                ImA = jnp.where(lane == 0, 0.0, ImA)
            else:
                nyq = jnp.concatenate([pltpu.roll(rt, (128-4*(g+4*i)) % 128, 1) if (g+4*i) else rt
                                       for i in range(8)], axis=0)
                ImA = jnp.where(lane == 0, nyq, ImA)
            if p4:
                Z1 = pltpu.roll(ImA, 1, 1); G_ = jnp.where(odd, ReA, Z1); E_ = jnp.where(odd, Z1, ReA)
                W1 = pltpu.roll(ImB, 1, 1); H4 = jnp.where(odd, ReB, W1); F2 = jnp.where(odd, W1, ReB)
                H_ = pltpu.roll(H4, 4, 1); Fm = pltpu.roll(F2, 2, 1)
                ins = (jnp.where(lo, E_, Fm).astype(bf16), jnp.where(lo, Fm, E_).astype(bf16),
                       jnp.where(mG, G_, H_).astype(bf16), jnp.where(mG, H_, G_).astype(bf16))
            else:
                Z0 = ReA; Z1 = pltpu.roll(ImA, 1, 1); Z2 = pltpu.roll(ReB, 2, 1); Z3 = pltpu.roll(ImB, 3, 1)
                O1 = jnp.where(odd, Z0, Z1); E_ = jnp.where(odd, Z1, Z0)
                O2 = jnp.where(odd, Z2, Z3); Fm = jnp.where(odd, Z3, Z2)
                ins = (jnp.where(lo, E_, Fm).astype(bf16), jnp.where(lo, Fm, E_).astype(bf16),
                       jnp.concatenate([O1, O2], axis=1).astype(bf16))
            yield
            q0 = _dot(ins[0], c2(I_N0)); q2 = _dot(ins[1], c2(I_N2))
            if p4:
                vp = _dot(ins[2], q4(2)); vm = _dot(ins[3], q4(3))
            else:
                qq = _dot(ins[2], n1())
            yield
            if p4:
                sv = vp+vm; dl = (vp-vm) * RS2
                dr = pltpu.roll(dl, 64, 1)
                qb = jnp.where(lo64, sv, dr+dl); qd = jnp.where(lo64, pltpu.roll(sv, 64, 1), dl-dr)
            else:
                qb, qd = qq[:, :128], qq[:, 128:]
            e = q0+q2; f = q0-q2
            if late:
                rt = get_rt()
                alt = jnp.where(odd, -1.0/(S*D), 1.0/(S*D))
                nq = jnp.concatenate([jnp.broadcast_to(rt[:, 4*(g+4*i):4*(g+4*i)+1], (8, 128))
                                      for i in range(8)], axis=0) * alt
                e = e + nq; f = f + nq
            x1 = load_grp(g) + jnp.concatenate([e+qb, f+qd, e-qb, f-qd], axis=1)
            xa[slot, 64*g:64*(g+1), :] = x1
            zb[slot, 64*g:64*(g+1), :] = (layernorm1 if late else layernorm)(x1).astype(bf16)
            yield

    def ffn_gen(slot, res, wait=False, pin=None, fin=None):
        acc = None
        z = zb[slot]
        for c in range(NCH):
            if wait and c == WSPLIT:
                for w in range(3): bg_copy(1, w).wait()
            g = _dot(z, wg[:, c*FC:(c+1)*FC]); yield
            u = _dot(z, wu[:, c*FC:(c+1)*FC]); yield
            h = (g*u).astype(bf16)
            if pin is not None and c in PINC:
                tbuf[pin, 0:16, :] = h[0:16, :]
            if fin is not None and c == NCH-1:
                for g_ in range(4):
                    fin(g_, acc[64*g_:64*(g_+1)] + _dot(h[64*g_:64*(g_+1)], wd[c*FC:(c+1)*FC, :]))
                yield
                return
            d = _dot(h, wd[c*FC:(c+1)*FC, :])
            acc = d if acc is None else acc + d
            yield
        res.append(acc)
    n_main = 3*NCH

    def column_gen():
        for k1 in [b_ + 8*a_ for b_ in range(8) for a_ in range(4)]:
            X = _dot(gm[k1], obuf[k1])
            xr, xi = X[:64], X[64:]
            off = (k1 >> 2)*256 + (k1 & 3)
            wrr = jnp.concatenate([wtab[0, 0, pl.ds(off, 64, stride=4), :],
                                   wtab[0, 1, pl.ds(off, 64, stride=4), :]], axis=1)
            wii = jnp.concatenate([wtab[1, 0, pl.ds(off, 64, stride=4), :],
                                   wtab[1, 1, pl.ds(off, 64, stride=4), :]], axis=1)
            Y = jnp.concatenate([xr*wrr - xi*wii, xr*wii + xi*wrr], axis=0).astype(bf16)
            tbuf[k1] = lax.dot_general(gm[k1], Y, (((0,), (0,)), ((), ())),
                                       preferred_element_type=f32).astype(bf16)
            if k1 >= 24: yield

    def nyq_gen():
        V = jnp.concatenate([vbuf[0], vbuf[1]], axis=0).astype(bf16)
        A1r = _dot(V, c2(I_C128)); A1i = -_dot(V, c2(I_S128))
        twc, tws = tw(0), tw(1)
        A2 = jnp.concatenate([A1r*twc + A1i*tws, A1i*twc - A1r*tws], axis=0).astype(bf16)
        yield
        Xn = _dot(_ub(cn[64*I_F16:64*I_F16+16, :])[:, 0:32], A2)
        wnr, wni = wn[0], wn[1]
        Yn = jnp.concatenate([Xn[:16]*wnr - Xn[16:]*wni, Xn[:16]*wni + Xn[16:]*wnr], axis=0).astype(bf16)
        yield
        B2 = _dot(_ub(cn[64*I_F16+16:64*I_F16+32, :])[:, 0:32], Yn)
        B1r = (B2[:16]*twc - B2[16:]*tws).astype(bf16); B1i = (B2[16:]*twc + B2[:16]*tws).astype(bf16)
        yield
        r = _dot(B1r, c2(I_C128)) - _dot(B1i, c2(I_S128))
        rbuf[0] = r[:8]; rbuf[1] = r[8:]
        yield

    def wprep_gen(p, q):
        pm = c1(I_P)
        for c in range(4*q, 4*q+4):
            blk = lax.dot_general(pm, wt[p, 0:256, 128*c:128*(c+1)], (((1,), (1,)), ((), ())),
                                  preferred_element_type=f32)
            for b in range(2):
                for a in range(8):
                    wtab[p, b, 256*a+16*c:256*a+16*c+16, :] = blk[16*a:16*a+16, 128*b:128*(b+1)]
            wn[p, c:c+1, :] = wt[p, 256:257, 128*c:128*(c+1)].astype(f32)
            yield

    def wq(q):
        yield from wprep_gen(0, q)
        yield from wprep_gen(1, q)

    def load_xin(j, g):
        return jnp.concatenate([xin[j, g+4*i].astype(f32) for i in range(8)], axis=0)
    stats = {}

    def ln_stage(j):
        x = jnp.concatenate([load_xin(j, g) for g in range(4)], axis=0)
        sx_, _, r = ln_stats(x)
        for g in range(4):
            stats[j, g] = (sx_[64*g:64*(g+1)], r[64*g:64*(g+1)])
        z0, z1, z2, z3 = [x[:, 128*i:128*(i+1)] for i in range(4)]
        a = z0+z2; b = z0-z2; c = z1+z3; dd = z1-z3
        yb[j & 1] = jnp.concatenate([a+c, a-c, b, dd], axis=1).astype(bf16)
        yield

    def dft_stage(j):
        slot = j & 1
        vt = jnp.zeros((8, 128), f32)
        for g in range(4):
            yy = yb[slot, 64*g:64*(g+1), :]
            y0 = yy[:, 0:128]; y2 = yy[:, 128:256]; bd = yy[:, 256:512]
            p0 = _dot(y0, c1(I_M0)); p2 = _dot(y2, c1(I_M2)); O = _dot(bd, m1())
            yield
            O1, O2 = O[:, :128], O[:, 128:]
            E_ = jnp.where(lo, p0, p2); Fm = jnp.where(lo, p2, p0)
            ReA = jnp.where(odd, O1, E_)
            ImA = pltpu.roll(jnp.where(odd, E_, O1), 127, 1)
            ReB = pltpu.roll(jnp.where(odd, O2, Fm), 126, 1)
            ImB = pltpu.roll(jnp.where(odd, Fm, O2), 125, 1)
            sx_, r = stats[j, g]
            ReA = (ReA - jnp.where(lane == 0, sx_, 0.0)) * r
            ImA = ImA * r; ReB = ReB * r; ImB = ImB * r
            for i in range(8):
                s1 = g + 4*i
                blk = ImA[8*i:8*i+8]
                vt = jnp.where(lane8 == 4*s1, pltpu.roll(blk, 4*s1, 1) if s1 else blk, vt)
            ImA = jnp.where(lane == 0, 0.0, ImA)
            yield
            for lb, (re, im) in enumerate(((ReA, ImA), (ReB, ImB))):
                r = fft_list([(re[8*i:8*i+8], im[8*i:8*i+8]) for i in range(8)], +1)
                for kp in range(8):
                    t = cmul_const(r[kp], kp*g, 32)
                    midp[slot, 0, lb, kp, g] = t[0]; midp[slot, 1, lb, kp, g] = t[1]
                yield
        if j >> 1: vt = pltpu.roll(vt, j >> 1, 1)
        vbuf[j & 1] = jnp.where((lane8 & 3) == (j >> 1), vt, vbuf[j & 1])

    def r4_stage(j):
        slot = j & 1
        for kp in range(8):
            outs = [fft_list([(midp[slot, 0, lb, kp, g], midp[slot, 1, lb, kp, g]) for g in range(4)], +1)
                    for lb in range(2)]
            for kq in range(4):
                re = jnp.concatenate([outs[0][kq][0], outs[1][kq][0]], axis=1)
                im = jnp.concatenate([outs[0][kq][1], outs[1][kq][1]], axis=1)
                obuf[kp+8*kq, 16*j:16*j+16, :] = jnp.concatenate([re, im], axis=0).astype(bf16)
            yield

    def stage(sidx, extra=()):
        gens = []
        if 0 <= sidx-1 < NT: gens.append(dft_stage(sidx-1))
        if sidx < NT: gens.append(ln_stage(sidx))
        if 0 <= sidx-2 < NT: gens.append(r4_stage(sidx-2))
        mix(*gens, *extra)

    x_copy(0).wait()
    stage(0); ggen_part(GSPLIT, 32)
    ccm.wait(); x_copy(1).wait()
    stage(1)
    x_copy(2).wait(); x_copy(3).wait()
    stage(2); stage(3)
    x_copy(4).wait(); x_copy(5).wait()
    stage(4); stage(5)
    x_copy(6).wait(); x_copy(7).wait(); w_copy(0, 0).wait(); w_copy(1, 0).wait()
    stage(6, (wq(0),))
    w_copy(0, 1).wait(); w_copy(1, 1).wait()
    stage(7, (wq(1),))
    for q in (2, 3):
        w_copy(0, q).wait(); w_copy(1, q).wait()
    ccn.wait()
    ny1 = nyq_gen()
    stage(8, (wq(2),)); stage(9, (wq(3),))
    next(ny1); next(ny1)

    def mk_inv(ja, slot, from_xin, late=False):
        ld = (lambda g: load_xin(ja, g)) if from_xin else (lambda g: xs[ja, 64*g:64*(g+1), :])
        return inv_gen(ja, ld, slot, late)

    def mk_fwd(jc, post=False):
        return fwd_gen(jc, lambda g: xs[jc, 64*g:64*(g+1), :], post, p4=not post, gp=1 if post else 2)

    def pin_idx(j):
        return None if isinstance(j, int) else 32 + (j >> 3)

    def col_and_pro(from_xin, ny):
        inv = mk_inv(0, 0, from_xin, late=True)
        col = column_gen()
        for _ in range(8):
            next(col); next(inv)
        for _ in col: pass
        next(ny); next(inv); next(ny)
        for _ in inv: pass
        for _ in ny: pass

    col_and_pro(True, ny1)
    for w in range(3): bg_copy(0, w).wait()

    def p3_body(j, slot, do_c, wait=False):
        res = []
        sides = []
        if do_c: sides.append((mk_fwd(j-1), POS_C))
        sides.append((mk_inv(j+1 if isinstance(j, int) else (j+1) & 7, 1-slot, True), POS_A))
        interleave(ffn_gen(slot, res, wait, pin=pin_idx(j)), n_main, sides)
        xs[j] = res[0] + xa[slot]

    p3_body(0, 0, False, wait=True)

    def p3(j, _):
        p3_body(j, j & 1, True)
        return 0
    lax.fori_loop(1, NT, p3, 0)

    ny2 = nyq_gen()
    fw = mk_fwd(NT-1, True)
    for k in range(12):
        next(fw, None)
        if k in (8, 9): next(ny2)
    for _ in fw: pass
    col_and_pro(False, ny2)

    def p5_body(j, slot):
        def fin(g, a):
            x2 = a + xa[slot, 64*g:64*(g+1), :]
            for i in range(8):
                outb[j, g, i] = x2[8*i:8*i+8].astype(bf16)
            o_copy(j, g).start()
        interleave(ffn_gen(slot, [], pin=pin_idx(j), fin=fin), n_main,
                   [(mk_inv((j+1) & 7, 1-slot, False), POS_A)])

    def p5(i, _):
        p5_body(2*i, 0); p5_body(2*i+1, 1)
        return 0
    lax.fori_loop(0, NT // 2, p5, 0)
    for j in range(NT):
        for g in range(4): o_copy(j, g).wait()


@jax.jit
def pallas_interleave_layers__spectral_gfnet__glu_gated_bilinear__prompt_kernel(
        A_x, A_w_r, A_w_i, B_x, B_w_gate, B_w_up, B_w_down):
    consts = build_consts()
    x3 = A_x.reshape(32, 64, D)
    hbm = pl.BlockSpec(memory_space=pltpu.HBM)
    out = pl.pallas_call(
        kernel,
        out_shape=jax.ShapeDtypeStruct((8, 4, 64, D), bf16),
        in_specs=[hbm]*8,
        out_specs=hbm,
        scratch_shapes=[
            pltpu.VMEM((NT, 32, 8, D), bf16),
            pltpu.VMEM((NT, TM, D), f32),
            pltpu.VMEM((2, TM, D), f32),
            pltpu.VMEM((2, TM, D), bf16),
            pltpu.VMEM((2, 257, 2048), bf16),
            pltpu.VMEM((2, 2, 2048, 128), f32),
            pltpu.VMEM((2, 16, 128), f32),
            pltpu.VMEM((D, F), bf16), pltpu.VMEM((D, F), bf16), pltpu.VMEM((F, D), bf16),
            pltpu.VMEM((448, 128), u32), pltpu.VMEM((864, 128), u32),
            pltpu.VMEM((32, 128, 128), bf16),
            pltpu.VMEM((32, 128, 256), bf16),
            pltpu.VMEM((33, 128, 256), bf16),
            pltpu.VMEM((2, 8, 128), f32),
            pltpu.VMEM((2, 8, 128), f32),
            pltpu.VMEM((NT, 4, 8, 8, D), bf16),
            pltpu.VMEM((2, 2, 8, 4, 8, 128), f32),
            pltpu.VMEM((2, 2, 8, 4, 8, 128), f32),
            pltpu.VMEM((2, TM, D), bf16),
            pltpu.VMEM((2, 2, 2, 8, 4, 8, 128), f32),
            pltpu.VMEM((3, 64, 128), f32),
            pltpu.SemaphoreType.DMA((NT,)), pltpu.SemaphoreType.DMA((2,)), pltpu.SemaphoreType.DMA((8,)),
            pltpu.SemaphoreType.DMA((6,)), pltpu.SemaphoreType.DMA((4*NT,)),
        ],
        compiler_params=pltpu.CompilerParams(vmem_limit_bytes=100*1024*1024),
    )(x3, A_w_r.T, A_w_i.T, B_w_gate, B_w_up, B_w_down, *consts)
    return out.reshape(1, S, D)
```

```python
import math

import ml_dtypes
import numpy as np
import jax
import jax.numpy as jnp
from jax import lax
from jax.experimental import pallas as pl
from jax.experimental.pallas import tpu as pltpu

BF = ml_dtypes.bfloat16
EPS = 1e-5
S, D, F = 2048, 512, 1792
NT, TM = 8, 256
FC = 256
NCH = F // FC
HB = F // 2
WSPLIT = 3
f32, bf16, i32, u32 = jnp.float32, jnp.bfloat16, jnp.int32, jnp.uint32

POS_C = [0, 1, 2, 3, 4, 5, 6, 7, 8, 8, 9, 9]
POS_A = [2, 5, 8, 11, 11, 12, 12, 13, 14, 14, 15, 16, 16, 17, 18, 18]
PINC = (0, 1, 2, 3)
GSPLIT = 8

I_M0, I_M2, I_P = 0, 1, 2
I_N0, I_N2, I_C128, I_S128, I_F16 = 0, 1, 2, 3, 4


def build_consts():
    d2 = np.arange(128)[:, None].astype(np.float64)

    def cs(l):
        ph = 2*np.pi*((d2*np.asarray(l)[None, :]) % 512)/512.0
        return np.cos(ph), np.sin(ph)
    m = np.arange(32)
    M0 = np.zeros((128, 128)); M2 = np.zeros((128, 128))
    co, si = cs(4*m);        M0[:, 4*m+0] = co; M0[:, 4*m+1] = -si
    M0[:, 1] = (-1.0)**np.arange(128)
    co, si = cs(128+4*m);    M0[:, 4*m+2] = co; M0[:, 4*m+3] = -si
    co, si = cs(4*m+2);      M2[:, 4*m+2] = co; M2[:, 4*m+3] = -si
    co, si = cs(128+4*m+2);  M2[:, (4*m+4) % 128] = co; M2[:, (4*m+5) % 128] = -si
    M1 = np.zeros((256, 256))
    t = np.arange(1, 128, 2)

    def odd_cols(l):
        co, si = cs(l)
        sg = np.where(l % 4 == 1, 1.0, -1.0)[None, :]
        return np.concatenate([co, -sg*si], axis=0), np.concatenate([-si, -sg*co], axis=0)
    re, im = odd_cols(t);      M1[:, t] = re;                 M1[:, (t+1) % 128] = im
    re, im = odd_cols(128+t);  M1[:, 128+(t+2) % 128] = re;   M1[:, 128+(t+3) % 128] = im
    sc = 1.0/(S*D)
    N0 = np.zeros((128, 128)); N2 = np.zeros((128, 128)); N1 = np.zeros((256, 256))

    def inv_rows(l, cl):
        co, si = cs(l)
        return (cl*co).T*sc, (-cl*si).T*sc
    cl0 = np.where(4*m == 0, 1.0, 2.0)[None, :]
    r_, i_ = inv_rows(4*m, cl0);       N0[4*m+0] = r_; N0[4*m+1] = i_
    N0[1] = (-1.0)**np.arange(128)*sc
    r_, i_ = inv_rows(128+4*m, 2.0);   N0[4*m+2] = r_; N0[4*m+3] = i_
    r_, i_ = inv_rows(4*m+2, 2.0);     N2[4*m+2] = r_; N2[4*m+3] = i_
    r_, i_ = inv_rows(128+4*m+2, 2.0); N2[(4*m+4) % 128] = r_; N2[(4*m+5) % 128] = i_

    def odd_rows(l):
        co, si = cs(l)
        sg = np.where(l % 4 == 1, 1.0, -1.0)[None, :]
        return (np.concatenate([2*co, -2*sg*si], axis=0).T*sc,
                np.concatenate([-2*si, -2*sg*co], axis=0).T*sc)
    re, im = odd_rows(t);      N1[t] = re;               N1[(t+1) % 128] = im
    re, im = odd_rows(128+t);  N1[128+(t+2) % 128] = re; N1[128+(t+3) % 128] = im
    a = np.arange(128)
    ph = 2*np.pi*((a[:, None]*a[None, :]) % 128)/128.0
    C128, S128 = np.cos(ph), np.sin(ph)
    sa = np.arange(16)[:, None]; kl = np.arange(128)[None, :]
    ph = 2*np.pi*(sa*kl)/2048.0
    tw = np.stack([np.cos(ph), np.sin(ph)]).astype(np.float32)
    b = np.arange(16)
    ph = 2*np.pi*((b[:, None]*b[None, :]) % 16)/16.0
    C, Sn = np.cos(ph), np.sin(ph)
    F16 = np.zeros((128, 128))
    F16[0:32, 0:32] = np.block([[C, Sn], [-Sn, C]]); F16[32:64, 0:32] = np.block([[C, -Sn], [Sn, C]])
    P = np.zeros((128, 128))
    for a_ in range(8):
        for k2lo in range(4):
            for k1lo in range(4):
                P[16*a_+4*k2lo+k1lo, 32*k2lo+4*a_+k1lo] = 1.0
    d3 = np.arange(64).astype(np.float64)
    Q = {1: np.zeros((128, 128)), -1: np.zeros((128, 128))}
    for lp in range(1, 256, 2):
        l, sg = (lp, 1.0) if lp % 4 == 1 else (512 - lp, -1.0)
        ph = 2*np.pi*((d3*l) % 512)/512.0
        co, si = np.cos(ph), np.sin(ph)
        t_ = lp % 128 + (0 if lp < 128 else 4)
        Qc = Q[1 if l % 8 == 1 else -1]
        Qc[:, t_ % 128] = np.concatenate([co, -si])
        Qc[:, (t_+1) % 128] = sg*np.concatenate([-si, -co])

    def pack(a):
        u = np.ascontiguousarray(a).view(np.uint16).astype(np.uint32)
        return (u[..., 0::2, :] | (u[..., 1::2, :] << 16)).astype(np.uint32)
    c1 = np.stack([M0, M2, P]).astype(BF)
    c2 = np.stack([N0, N2, C128, S128, F16]).astype(BF)
    q4 = np.stack([Q[1], Q[-1], 2*sc*Q[1].T, 2*sc*Q[-1].T]).astype(BF)
    pm1 = pack(M1.astype(BF)); pn1 = pack(N1.astype(BF))
    cm = np.concatenate([pack(c1).reshape(192, 128), pm1[:, :128], pm1[:, 128:]], axis=0)
    cn = np.concatenate([pack(c2).reshape(320, 128), pn1[:, :128], pn1[:, 128:],
                         tw.reshape(32, 128).view(np.uint32), pack(q4).reshape(256, 128)], axis=0)
    return cm, cn


def _ub(v):
    return pltpu.bitcast(v, bf16)


def _dot(a, b):
    return jnp.dot(a, b, preferred_element_type=f32)


def cmul_const(v, num, den):
    re, im = v
    n = num % den
    if n == 0: return (re, im)
    if 4*n == den: return (im, -re)
    if 2*n == den: return (-re, -im)
    if 4*n == 3*den: return (-im, re)
    c = math.cos(2*math.pi*n/den); s = -math.sin(2*math.pi*n/den)
    if (8*n) % den == 0:
        r = math.sqrt(0.5)
        sc = 1.0 if c > 0 else -1.0; ss = 1.0 if s > 0 else -1.0
        a = (re - im) if sc*ss > 0 else (re + im)
        b = (re + im) if sc*ss > 0 else (im - re)
        return (a*(sc*r), b*(sc*r))
    return (re*c - im*s, re*s + im*c)


def cadd(a, b): return (a[0]+b[0], a[1]+b[1])
def csub(a, b): return (a[0]-b[0], a[1]-b[1])


def fft_list(v, sign):
    n = len(v)
    if n == 2: return [cadd(v[0], v[1]), csub(v[0], v[1])]
    if n == 4:
        a = cadd(v[0], v[2]); b = csub(v[0], v[2]); c = cadd(v[1], v[3]); d = csub(v[1], v[3])
        dj = (d[1], -d[0]) if sign > 0 else (-d[1], d[0])
        return [cadd(a, c), cadd(b, dj), csub(a, c), csub(b, dj)]
    e = fft_list(v[0::2], sign); o = fft_list(v[1::2], sign)
    out = [None]*n
    for k in range(n//2):
        t = cmul_const(o[k], sign*k, n)
        out[k] = cadd(e[k], t); out[k+n//2] = csub(e[k], t)
    return out


def layernorm(x):
    m = jnp.mean(x, axis=-1, keepdims=True)
    xc = x - m
    v = jnp.mean(xc*xc, axis=-1, keepdims=True)
    return xc * lax.rsqrt(v + EPS)


def ln_stats(x):
    s1 = jnp.sum(x, axis=-1, keepdims=True)
    s2 = jnp.sum(x*x, axis=-1, keepdims=True)
    m = s1 * (1.0/D)
    v = jnp.maximum(s2 * (1.0/D) - m*m, 0.0)
    return s1, m, lax.rsqrt(v + EPS)


def layernorm1(x):
    _, m, r = ln_stats(x)
    return x*r - m*r


def run(gen):
    for _ in gen: pass


def mix(*gens):
    alive = list(gens)
    while alive:
        for g in list(alive):
            if next(g, 'end') == 'end': alive.remove(g)


def interleave(main, nmain, sides):
    st = [[g, list(p), 0] for g, p in sides]

    def emit(step):
        for e in st:
            while e[2] < len(e[1]) and e[1][e[2]] <= step:
                next(e[0], None)
                e[2] += 1
    emit(-1)
    for i in range(nmain):
        next(main)
        emit(i)
    for _ in main: pass
    for e in st:
        for _ in e[0]: pass


def kernel(x_hbm, wr_hbm, wi_hbm, wg_hbm, wu_hbm, wd_hbm, cm_hbm, cn_hbm,
           out_hbm,
           xin, xs, xa, zb, wt, wtab, wn, wg, wu, wd, cm, cn, gm, obuf, tbuf, vbuf, rbuf, outb,
           midc, mida, yb, midp, gt,
           sx, sc, sw, sb, so):
    lane = lax.broadcasted_iota(i32, (64, 128), 1)
    odd = (lane & 1) == 1
    lo = (lane & 3) < 2
    lane8 = lax.broadcasted_iota(i32, (8, 128), 1)
    lo64 = lane < 64
    l8 = lane & 7
    mG = (l8 <= 2) | (l8 == 7)
    RS2 = math.sqrt(0.5)

    def aligned(j, k):
        return k*j if isinstance(j, int) else pl.multiple_of(k*j, k)

    def x_copy(j):
        return pltpu.make_async_copy(x_hbm.at[:, pl.ds(aligned(j, 8), 8), :], xin.at[j], sx.at[j])
    ccm = pltpu.make_async_copy(cm_hbm, cm, sc.at[0])
    ccn = pltpu.make_async_copy(cn_hbm, cn, sc.at[1])

    def w_copy(p):
        return pltpu.make_async_copy((wr_hbm, wi_hbm)[p], wt.at[p], sw.at[p])

    def bg_copy(h, which):
        o = HB*h if isinstance(h, int) else pl.multiple_of(HB*h, 128)
        if which == 0:
            return pltpu.make_async_copy(wg_hbm.at[:, pl.ds(o, HB)], wg.at[:, pl.ds(o, HB)], sb.at[3*h])
        if which == 1:
            return pltpu.make_async_copy(wu_hbm.at[:, pl.ds(o, HB)], wu.at[:, pl.ds(o, HB)], sb.at[3*h+1])
        return pltpu.make_async_copy(wd_hbm.at[pl.ds(o, HB), :], wd.at[pl.ds(o, HB), :], sb.at[3*h+2])

    def o_copy(j, g):
        return pltpu.make_async_copy(outb.at[j, g], out_hbm.at[:, g, pl.ds(aligned(j, 8), 8), :], so.at[4*j+g])

    def c1(i): return _ub(cm[64*i:64*(i+1), :])
    def m1(): return jnp.concatenate([_ub(cm[192:320, :]), _ub(cm[320:448, :])], axis=1)
    def c2(i): return _ub(cn[64*i:64*(i+1), :])
    def n1(): return jnp.concatenate([_ub(cn[320:448, :]), _ub(cn[448:576, :])], axis=1)
    def q4(i): return _ub(cn[608+64*i:608+64*(i+1), :])
    def tw(i): return pltpu.bitcast(cn[576+16*i:576+16*(i+1), :], f32)

    x_copy(0).start()
    ccm.start()

    def _sx(j, _):
        x_copy(j).start(); return 0
    lax.fori_loop(1, NT, _sx, 0)

    w_copy(0).start()
    w_copy(1).start()
    ccn.start()

    def _sb(h, _):
        for w in range(3): bg_copy(h, w).start()
        return 0
    lax.fori_loop(0, 2, _sb, 0)

    def ggen_tables():
        r64 = lax.broadcasted_iota(i32, (64, 128), 0); c64 = lax.broadcasted_iota(i32, (64, 128), 1)
        s2c = 8*(c64 >> 4) + (c64 & 7)
        pc0 = ((c64 >> 3) & 1) == 0
        th = ((r64*s2c) & 63).astype(f32) * (2*math.pi/64)
        c0 = jnp.cos(th); s0 = jnp.sin(th)
        gt[0] = jnp.where(pc0, c0, s0); gt[1] = jnp.where(pc0, -s0, c0)
        k1r = lax.broadcasted_iota(i32, (32, 128), 0); c32 = lax.broadcasted_iota(i32, (32, 128), 1)
        ph = (k1r*(8*(c32 >> 4) + (c32 & 7))).astype(f32) * (2*math.pi/2048)
        gt[2, 0:32] = jnp.cos(ph); gt[2, 32:64] = jnp.sin(ph)

    def ggen_part(lo_, hi_):
        A0t = gt[0]; A0b = gt[1]
        for k1 in range(lo_, hi_):
            cv = gt[2, k1:k1+1]; sv = gt[2, 32+k1:33+k1]
            gm[k1, 0:64, :] = (A0t*cv + A0b*sv).astype(bf16)
            gm[k1, 64:128, :] = (A0b*cv - A0t*sv).astype(bf16)

    ggen_tables()
    ggen_part(0, GSPLIT)
    vbuf[...] = jnp.zeros(vbuf.shape, f32)

    def fwd_gen(j, load_grp, post, p4, gp):
        vt = jnp.zeros((8, 128), f32)
        cat = lambda l: l[0] if len(l) == 1 else jnp.concatenate(l, axis=0)
        for g0 in range(0, 4, gp):
            ins = []; sts = []
            for g in range(g0, g0+gp):
                x = load_grp(g)
                if post:
                    sx_, _, r = ln_stats(x); sts.append((sx_, r))
                else:
                    x = layernorm(x)
                z0, z1, z2, z3 = [x[:, 128*i:128*(i+1)] for i in range(4)]
                a = z0+z2; b = z0-z2; c = z1+z3; dd = z1-z3
                y0 = (a+c).astype(bf16); y2 = (a-c).astype(bf16)
                if p4:
                    T1 = jnp.where(lo64, b, pltpu.roll(dd, 64, 1))
                    T2 = jnp.where(lo64, pltpu.roll(b-dd, 64, 1), b+dd) * RS2
                    ins.append((y0, y2, (T1+T2).astype(bf16), (T1-T2).astype(bf16)))
                else:
                    ins.append((y0, y2, jnp.concatenate([b, dd], axis=1).astype(bf16)))
                yield
            P0 = _dot(cat([t[0] for t in ins]), c1(I_M0)); P2 = _dot(cat([t[1] for t in ins]), c1(I_M2))
            if p4:
                PP = _dot(cat([t[2] for t in ins]), q4(0)); PM = _dot(cat([t[3] for t in ins]), q4(1))
            else:
                OO = _dot(cat([t[2] for t in ins]), m1())
            for g in range(g0, g0+gp):
                sl = slice(64*(g-g0), 64*(g-g0+1))
                p0, p2 = P0[sl], P2[sl]
                E_ = jnp.where(lo, p0, p2); Fm = jnp.where(lo, p2, p0)
                if p4:
                    Pp, Pm = PP[sl], PM[sl]
                    G_ = jnp.where(mG, Pp, Pm); H_ = jnp.where(mG, Pm, Pp)
                    ReA = jnp.where(odd, G_, E_)
                    ImA = pltpu.roll(jnp.where(odd, E_, G_), 127, 1)
                    H4 = pltpu.roll(H_, 124, 1); F2 = pltpu.roll(Fm, 126, 1)
                    ReB = jnp.where(odd, H4, F2)
                    ImB = pltpu.roll(jnp.where(odd, F2, H4), 127, 1)
                else:
                    O1, O2 = OO[sl, :128], OO[sl, 128:]
                    ReA = jnp.where(odd, O1, E_)
                    ImA = pltpu.roll(jnp.where(odd, E_, O1), 127, 1)
                    ReB = pltpu.roll(jnp.where(odd, O2, Fm), 126, 1)
                    ImB = pltpu.roll(jnp.where(odd, Fm, O2), 125, 1)
                if post:
                    sx_, r = sts[g-g0]
                    ReA = (ReA - jnp.where(lane == 0, sx_, 0.0)) * r
                    ImA = ImA * r; ReB = ReB * r; ImB = ImB * r
                for i in range(8):
                    s1 = g + 4*i
                    blk = ImA[8*i:8*i+8]
                    vt = jnp.where(lane8 == 4*s1, pltpu.roll(blk, 4*s1, 1) if s1 else blk, vt)
                ImA = jnp.where(lane == 0, 0.0, ImA)
                for lb, (re, im) in enumerate(((ReA, ImA), (ReB, ImB))):
                    r = fft_list([(re[8*i:8*i+8], im[8*i:8*i+8]) for i in range(8)], +1)
                    for kp in range(8):
                        t = cmul_const(r[kp], kp*g, 32)
                        midc[0, lb, kp, g] = t[0]; midc[1, lb, kp, g] = t[1]
                yield
        vt = pltpu.roll(vt, j >> 1, 1)
        h = j & 1
        vbuf[h] = jnp.where((lane8 & 3) == (j >> 1), vt, vbuf[h])
        r0 = aligned(j, 16)
        for kp in range(8):
            outs = [fft_list([(midc[0, lb, kp, g], midc[1, lb, kp, g]) for g in range(4)], +1) for lb in range(2)]
            for kq in range(4):
                re = jnp.concatenate([outs[0][kq][0], outs[1][kq][0]], axis=1)
                im = jnp.concatenate([outs[0][kq][1], outs[1][kq][1]], axis=1)
                obuf[kp+8*kq, pl.ds(r0, 16), :] = jnp.concatenate([re, im], axis=0).astype(bf16)
            if kp % 2 == 1: yield

    def inv_gen(j, load_grp, slot, late):
        p4 = not late
        r0 = aligned(j, 16)
        for b in range(8):
            ts = [tbuf[8*a+b, pl.ds(r0, 16), :].astype(f32) for a in range(4)]
            for lb in range(2):
                r = fft_list([(t[:8, 128*lb:128*(lb+1)], t[8:, 128*lb:128*(lb+1)]) for t in ts], -1)
                for g in range(4):
                    t = cmul_const(r[g], -g*b, 32)
                    mida[0, lb, b, g] = t[0]; mida[1, lb, b, g] = t[1]
            if b % 2 == 1 or late: yield

        def get_rt():
            rt = rbuf[j & 1]
            if isinstance(j, int):
                if j >> 1: rt = pltpu.roll(rt, 128 - (j >> 1), 1)
            else:
                rt = pltpu.roll(rt, (128 - (j >> 1)) & 127, 1)
            return rt
        if not late: rt = get_rt()
        for g in range(4):
            res = []
            for lb in range(2):
                r = fft_list([(mida[0, lb, b, g], mida[1, lb, b, g]) for b in range(8)], -1)
                res.append((jnp.concatenate([r[i][0] for i in range(8)], axis=0),
                            jnp.concatenate([r[i][1] for i in range(8)], axis=0)))
            (ReA, ImA), (ReB, ImB) = res
            if late:
                ImA = jnp.where(lane == 0, 0.0, ImA)
            else:
                nyq = jnp.concatenate([pltpu.roll(rt, (128-4*(g+4*i)) % 128, 1) if (g+4*i) else rt
                                       for i in range(8)], axis=0)
                ImA = jnp.where(lane == 0, nyq, ImA)
            if p4:
                Z1 = pltpu.roll(ImA, 1, 1); G_ = jnp.where(odd, ReA, Z1); E_ = jnp.where(odd, Z1, ReA)
                W1 = pltpu.roll(ImB, 1, 1); H4 = jnp.where(odd, ReB, W1); F2 = jnp.where(odd, W1, ReB)
                H_ = pltpu.roll(H4, 4, 1); Fm = pltpu.roll(F2, 2, 1)
                ins = (jnp.where(lo, E_, Fm).astype(bf16), jnp.where(lo, Fm, E_).astype(bf16),
                       jnp.where(mG, G_, H_).astype(bf16), jnp.where(mG, H_, G_).astype(bf16))
            else:
                Z0 = ReA; Z1 = pltpu.roll(ImA, 1, 1); Z2 = pltpu.roll(ReB, 2, 1); Z3 = pltpu.roll(ImB, 3, 1)
                O1 = jnp.where(odd, Z0, Z1); E_ = jnp.where(odd, Z1, Z0)
                O2 = jnp.where(odd, Z2, Z3); Fm = jnp.where(odd, Z3, Z2)
                ins = (jnp.where(lo, E_, Fm).astype(bf16), jnp.where(lo, Fm, E_).astype(bf16),
                       jnp.concatenate([O1, O2], axis=1).astype(bf16))
            yield
            q0 = _dot(ins[0], c2(I_N0)); q2 = _dot(ins[1], c2(I_N2))
            if p4:
                vp = _dot(ins[2], q4(2)); vm = _dot(ins[3], q4(3))
            else:
                qq = _dot(ins[2], n1())
            yield
            if p4:
                sv = vp+vm; dl = (vp-vm) * RS2
                dr = pltpu.roll(dl, 64, 1)
                qb = jnp.where(lo64, sv, dr+dl); qd = jnp.where(lo64, pltpu.roll(sv, 64, 1), dl-dr)
            else:
                qb, qd = qq[:, :128], qq[:, 128:]
            e = q0+q2; f = q0-q2
            if late:
                rt = get_rt()
                alt = jnp.where(odd, -1.0/(S*D), 1.0/(S*D))
                nq = jnp.concatenate([jnp.broadcast_to(rt[:, 4*(g+4*i):4*(g+4*i)+1], (8, 128))
                                      for i in range(8)], axis=0) * alt
                e = e + nq; f = f + nq
            x1 = load_grp(g) + jnp.concatenate([e+qb, f+qd, e-qb, f-qd], axis=1)
            xa[slot, 64*g:64*(g+1), :] = x1
            zb[slot, 64*g:64*(g+1), :] = (layernorm1 if late else layernorm)(x1).astype(bf16)
            yield

    def ffn_gen(slot, res, wait=False, pin=None, fin=None):
        acc = None
        z = zb[slot]
        for c in range(NCH):
            if wait and c == WSPLIT:
                for w in range(3): bg_copy(1, w).wait()
            g = _dot(z, wg[:, c*FC:(c+1)*FC]); yield
            u = _dot(z, wu[:, c*FC:(c+1)*FC]); yield
            h = (g*u).astype(bf16)
            if pin is not None and c in PINC:
                tbuf[pin, 0:16, :] = h[0:16, :]
            if fin is not None and c == NCH-1:
                for g_ in range(4):
                    fin(g_, acc[64*g_:64*(g_+1)] + _dot(h[64*g_:64*(g_+1)], wd[c*FC:(c+1)*FC, :]))
                yield
                return
            d = _dot(h, wd[c*FC:(c+1)*FC, :])
            acc = d if acc is None else acc + d
            yield
        res.append(acc)
    n_main = 3*NCH

    def column_gen():
        for k1 in [b_ + 8*a_ for b_ in range(8) for a_ in range(4)]:
            X = _dot(gm[k1], obuf[k1])
            xr, xi = X[:64], X[64:]
            off = (k1 >> 2)*256 + (k1 & 3)
            wrr = jnp.concatenate([wtab[0, 0, pl.ds(off, 64, stride=4), :],
                                   wtab[0, 1, pl.ds(off, 64, stride=4), :]], axis=1)
            wii = jnp.concatenate([wtab[1, 0, pl.ds(off, 64, stride=4), :],
                                   wtab[1, 1, pl.ds(off, 64, stride=4), :]], axis=1)
            Y = jnp.concatenate([xr*wrr - xi*wii, xr*wii + xi*wrr], axis=0).astype(bf16)
            tbuf[k1] = lax.dot_general(gm[k1], Y, (((0,), (0,)), ((), ())),
                                       preferred_element_type=f32).astype(bf16)
            if k1 >= 24: yield

    def nyq_gen():
        V = jnp.concatenate([vbuf[0], vbuf[1]], axis=0).astype(bf16)
        A1r = _dot(V, c2(I_C128)); A1i = -_dot(V, c2(I_S128))
        twc, tws = tw(0), tw(1)
        A2 = jnp.concatenate([A1r*twc + A1i*tws, A1i*twc - A1r*tws], axis=0).astype(bf16)
        yield
        Xn = _dot(_ub(cn[64*I_F16:64*I_F16+16, :])[:, 0:32], A2)
        wnr, wni = wn[0], wn[1]
        Yn = jnp.concatenate([Xn[:16]*wnr - Xn[16:]*wni, Xn[:16]*wni + Xn[16:]*wnr], axis=0).astype(bf16)
        yield
        B2 = _dot(_ub(cn[64*I_F16+16:64*I_F16+32, :])[:, 0:32], Yn)
        B1r = (B2[:16]*twc - B2[16:]*tws).astype(bf16); B1i = (B2[16:]*twc + B2[:16]*tws).astype(bf16)
        yield
        r = _dot(B1r, c2(I_C128)) - _dot(B1i, c2(I_S128))
        rbuf[0] = r[:8]; rbuf[1] = r[8:]
        yield

    def wprep_gen(p, q):
        pm = c1(I_P)
        for c in range(4*q, 4*q+4):
            blk = lax.dot_general(pm, wt[p, 0:256, 128*c:128*(c+1)], (((1,), (1,)), ((), ())),
                                  preferred_element_type=f32)
            for b in range(2):
                for a in range(8):
                    wtab[p, b, 256*a+16*c:256*a+16*c+16, :] = blk[16*a:16*a+16, 128*b:128*(b+1)]
            wn[p, c:c+1, :] = wt[p, 256:257, 128*c:128*(c+1)].astype(f32)
            yield

    def wq(p, h):
        yield from wprep_gen(p, 2*h)
        yield from wprep_gen(p, 2*h+1)

    def load_xin(j, g):
        return jnp.concatenate([xin[j, g+4*i].astype(f32) for i in range(8)], axis=0)
    stats = {}

    def ln_stage(j):
        x = jnp.concatenate([load_xin(j, g) for g in range(4)], axis=0)
        sx_, _, r = ln_stats(x)
        for g in range(4):
            stats[j, g] = (sx_[64*g:64*(g+1)], r[64*g:64*(g+1)])
        z0, z1, z2, z3 = [x[:, 128*i:128*(i+1)] for i in range(4)]
        a = z0+z2; b = z0-z2; c = z1+z3; dd = z1-z3
        yb[j & 1] = jnp.concatenate([a+c, a-c, b, dd], axis=1).astype(bf16)
        yield

    def dft_stage(j):
        slot = j & 1
        vt = jnp.zeros((8, 128), f32)
        for g in range(4):
            yy = yb[slot, 64*g:64*(g+1), :]
            y0 = yy[:, 0:128]; y2 = yy[:, 128:256]; bd = yy[:, 256:512]
            p0 = _dot(y0, c1(I_M0)); p2 = _dot(y2, c1(I_M2)); O = _dot(bd, m1())
            yield
            O1, O2 = O[:, :128], O[:, 128:]
            E_ = jnp.where(lo, p0, p2); Fm = jnp.where(lo, p2, p0)
            ReA = jnp.where(odd, O1, E_)
            ImA = pltpu.roll(jnp.where(odd, E_, O1), 127, 1)
            ReB = pltpu.roll(jnp.where(odd, O2, Fm), 126, 1)
            ImB = pltpu.roll(jnp.where(odd, Fm, O2), 125, 1)
            sx_, r = stats[j, g]
            ReA = (ReA - jnp.where(lane == 0, sx_, 0.0)) * r
            ImA = ImA * r; ReB = ReB * r; ImB = ImB * r
            for i in range(8):
                s1 = g + 4*i
                blk = ImA[8*i:8*i+8]
                vt = jnp.where(lane8 == 4*s1, pltpu.roll(blk, 4*s1, 1) if s1 else blk, vt)
            ImA = jnp.where(lane == 0, 0.0, ImA)
            yield
            for lb, (re, im) in enumerate(((ReA, ImA), (ReB, ImB))):
                r = fft_list([(re[8*i:8*i+8], im[8*i:8*i+8]) for i in range(8)], +1)
                for kp in range(8):
                    t = cmul_const(r[kp], kp*g, 32)
                    midp[slot, 0, lb, kp, g] = t[0]; midp[slot, 1, lb, kp, g] = t[1]
                yield
        if j >> 1: vt = pltpu.roll(vt, j >> 1, 1)
        vbuf[j & 1] = jnp.where((lane8 & 3) == (j >> 1), vt, vbuf[j & 1])

    def r4_stage(j):
        slot = j & 1
        for kp in range(8):
            outs = [fft_list([(midp[slot, 0, lb, kp, g], midp[slot, 1, lb, kp, g]) for g in range(4)], +1)
                    for lb in range(2)]
            for kq in range(4):
                re = jnp.concatenate([outs[0][kq][0], outs[1][kq][0]], axis=1)
                im = jnp.concatenate([outs[0][kq][1], outs[1][kq][1]], axis=1)
                obuf[kp+8*kq, 16*j:16*j+16, :] = jnp.concatenate([re, im], axis=0).astype(bf16)
            yield

    def stage(sidx, extra=()):
        gens = []
        if 0 <= sidx-1 < NT: gens.append(dft_stage(sidx-1))
        if sidx < NT: gens.append(ln_stage(sidx))
        if 0 <= sidx-2 < NT: gens.append(r4_stage(sidx-2))
        mix(*gens, *extra)

    x_copy(0).wait()
    stage(0); ggen_part(GSPLIT, 32)
    ccm.wait(); x_copy(1).wait()
    stage(1)
    x_copy(2).wait(); x_copy(3).wait()
    stage(2); stage(3)
    x_copy(4).wait(); x_copy(5).wait()
    stage(4); stage(5)
    x_copy(6).wait(); x_copy(7).wait(); w_copy(0).wait()
    stage(6, (wq(0, 0),))
    stage(7, (wq(0, 1),))
    w_copy(1).wait()
    ccn.wait()
    ny1 = nyq_gen()
    stage(8, (wq(1, 0),)); stage(9, (wq(1, 1),))
    next(ny1); next(ny1)

    def mk_inv(ja, slot, from_xin, late=False):
        ld = (lambda g: load_xin(ja, g)) if from_xin else (lambda g: xs[ja, 64*g:64*(g+1), :])
        return inv_gen(ja, ld, slot, late)

    def mk_fwd(jc, post=False):
        return fwd_gen(jc, lambda g: xs[jc, 64*g:64*(g+1), :], post, p4=not post, gp=1 if post else 2)

    def pin_idx(j):
        return None if isinstance(j, int) else 32 + (j >> 3)

    def col_and_pro(from_xin, ny):
        inv = mk_inv(0, 0, from_xin, late=True)
        col = column_gen()
        for _ in range(8):
            next(col); next(inv)
        for _ in col: pass
        next(ny); next(inv); next(ny)
        for _ in inv: pass
        for _ in ny: pass

    col_and_pro(True, ny1)
    for w in range(3): bg_copy(0, w).wait()

    def p3_body(j, slot, do_c, wait=False):
        res = []
        sides = []
        if do_c: sides.append((mk_fwd(j-1), POS_C))
        sides.append((mk_inv(j+1 if isinstance(j, int) else (j+1) & 7, 1-slot, True), POS_A))
        interleave(ffn_gen(slot, res, wait, pin=pin_idx(j)), n_main, sides)
        xs[j] = res[0] + xa[slot]

    p3_body(0, 0, False, wait=True)

    def p3(j, _):
        p3_body(j, j & 1, True)
        return 0
    lax.fori_loop(1, NT, p3, 0)

    ny2 = nyq_gen()
    fw = mk_fwd(NT-1, True)
    for k in range(12):
        next(fw, None)
        if k in (8, 9): next(ny2)
    for _ in fw: pass
    col_and_pro(False, ny2)

    def p5_body(j, slot):
        def fin(g, a):
            x2 = a + xa[slot, 64*g:64*(g+1), :]
            for i in range(8):
                outb[j, g, i] = x2[8*i:8*i+8].astype(bf16)
            o_copy(j, g).start()
        interleave(ffn_gen(slot, [], pin=pin_idx(j), fin=fin), n_main,
                   [(mk_inv((j+1) & 7, 1-slot, False), POS_A)])

    def p5(i, _):
        p5_body(2*i, 0); p5_body(2*i+1, 1)
        return 0
    lax.fori_loop(0, NT // 2, p5, 0)
    for j in range(NT):
        for g in range(4): o_copy(j, g).wait()


@jax.jit
def pallas_interleave_layers__spectral_gfnet__glu_gated_bilinear__prompt_kernel(
        A_x, A_w_r, A_w_i, B_x, B_w_gate, B_w_up, B_w_down):
    consts = build_consts()
    x3 = A_x.reshape(32, 64, D)
    hbm = pl.BlockSpec(memory_space=pltpu.HBM)
    out = pl.pallas_call(
        kernel,
        out_shape=jax.ShapeDtypeStruct((8, 4, 64, D), bf16),
        in_specs=[hbm]*8,
        out_specs=hbm,
        scratch_shapes=[
            pltpu.VMEM((NT, 32, 8, D), bf16),
            pltpu.VMEM((NT, TM, D), f32),
            pltpu.VMEM((2, TM, D), f32),
            pltpu.VMEM((2, TM, D), bf16),
            pltpu.VMEM((2, 257, 2048), bf16),
            pltpu.VMEM((2, 2, 2048, 128), f32),
            pltpu.VMEM((2, 16, 128), f32),
            pltpu.VMEM((D, F), bf16), pltpu.VMEM((D, F), bf16), pltpu.VMEM((F, D), bf16),
            pltpu.VMEM((448, 128), u32), pltpu.VMEM((864, 128), u32),
            pltpu.VMEM((32, 128, 128), bf16),
            pltpu.VMEM((32, 128, 256), bf16),
            pltpu.VMEM((33, 128, 256), bf16),
            pltpu.VMEM((2, 8, 128), f32),
            pltpu.VMEM((2, 8, 128), f32),
            pltpu.VMEM((NT, 4, 8, 8, D), bf16),
            pltpu.VMEM((2, 2, 8, 4, 8, 128), f32),
            pltpu.VMEM((2, 2, 8, 4, 8, 128), f32),
            pltpu.VMEM((2, TM, D), bf16),
            pltpu.VMEM((2, 2, 2, 8, 4, 8, 128), f32),
            pltpu.VMEM((3, 64, 128), f32),
            pltpu.SemaphoreType.DMA((NT,)), pltpu.SemaphoreType.DMA((2,)), pltpu.SemaphoreType.DMA((2,)),
            pltpu.SemaphoreType.DMA((6,)), pltpu.SemaphoreType.DMA((4*NT,)),
        ],
        compiler_params=pltpu.CompilerParams(vmem_limit_bytes=100*1024*1024),
    )(x3, A_w_r.T, A_w_i.T, B_w_gate, B_w_up, B_w_down, *consts)
    return out.reshape(1, S, D)
```
